```python
import jax
import jax.numpy as jnp

def _softmax(x, axis=-1):
    return jax.nn.softmax(x, axis=axis)
def _gelu(x):
    return jax.nn.gelu(x, approximate=True)
def _silu(x):
    return jax.nn.silu(x)
def _sigmoid(x):
    return jax.nn.sigmoid(x)
def _layernorm(x, axis=-1, eps=1e-5):
    m = jnp.mean(x, axis=axis, keepdims=True)
    v = jnp.var(x, axis=axis, keepdims=True)
    return (x - m) / jnp.sqrt(v + eps)
def _scatter_add(tgt, idx, src, axis=0):
    return tgt.at[idx].add(src)
def _segment_sum(src, seg, n):
    return jax.ops.segment_sum(src, seg, n)
class _Rng:
    def __init__(self, key):
        self._k = key
    def _next(self):
        self._k, sub = jax.random.split(self._k)
        return sub
    def normal(self, shape):
        return jax.random.normal(self._next(), shape, dtype=jnp.bfloat16)
    def randint(self, lo, hi, shape):
        return jax.random.randint(self._next(), shape, lo, hi, dtype=jnp.int32)
    def uniform(self, shape, lo=0.0, hi=1.0):
        return jax.random.uniform(self._next(), shape, jnp.bfloat16, lo, hi)
    def permutation(self, n):
        return jax.random.permutation(self._next(), n)


kernel_name = 'sequential_preLN__sliding_block_cached__glu_gated_swiglu__decode'

def setup_inputs():
    _rng = _Rng(jax.random.key(int.from_bytes(__import__("os").urandom(4), "little")))
    _w = (lambda a: (lambda t: t.astype(jnp.bfloat16) if jnp.issubdtype(t.dtype, jnp.floating) else t)(jnp.asarray(a)))
    def _A_setup():
        B, Sq, D = 1, 1, 640
        Hq, Hkv, Sk, Dh = 32, 32, 32768, 192
        assert Hq % Hkv == 0, (Hq, Hkv)
        return {
            "x": _w((lambda *s: _rng.normal(s) * 0.05)(B, Sq, D)),
            "k_cache": _w((lambda *s: _rng.normal(s) * 0.05)(B, Hkv, Sk, Dh)),
            "v_cache": _w((lambda *s: _rng.normal(s) * 0.05)(B, Hkv, Sk, Dh)),
            "wq": _w((lambda *s: _rng.normal(s) * 0.05)(D, Hq * Dh) * (D ** -0.5)),
            "wo": _w((lambda *s: _rng.normal(s) * 0.05)(Hq * Dh, D) * ((Hq * Dh) ** -0.5)),
        }
    _A_in = _A_setup()

    def _B_setup():
        B, S, D, F = 1, 1, 640, 1536
        return {
            "x": _w((lambda *s: _rng.normal(s) * 0.05)(B, S, D)),
            "w1": _w((lambda *s: _rng.normal(s) * 0.05)(D, F) * (2.0 / D) ** 0.5),
            "w3": _w((lambda *s: _rng.normal(s) * 0.05)(D, F) * (2.0 / D) ** 0.5),
            "w2": _w((lambda *s: _rng.normal(s) * 0.05)(F, D) * (2.0 / F) ** 0.5),
        }
    _B_in = _B_setup()

    return {
        "A_x": _A_in["x"],
        "A_k_cache": _A_in["k_cache"],
        "A_v_cache": _A_in["v_cache"],
        "A_wq": _A_in["wq"],
        "A_wo": _A_in["wo"],
        "B_x": _B_in["x"],
        "B_w1": _B_in["w1"],
        "B_w3": _B_in["w3"],
        "B_w2": _B_in["w2"],
    }

def reference(A_x, A_k_cache, A_v_cache, A_wq, A_wo, B_x, B_w1, B_w3, B_w2):
    def _A_ref(x, k_cache, v_cache, wq, wo):
        B, Sq, D = x.shape
        Hq, Dh = 32, 192
        Hkv, Sk = k_cache.shape[1], k_cache.shape[2]
        W = min(4096, max(256, Sk // 4))
        rep = Hq // Hkv
        q = (lambda x, *d: x.transpose(*d))((x @ wq).reshape(B, Sq, Hq, Dh), 0, 2, 1, 3)
        k = jnp.repeat(k_cache[:, :, Sk - W:, :], rep, axis=1)
        v = jnp.repeat(v_cache[:, :, Sk - W:, :], rep, axis=1)
        scores = jnp.einsum("bhqd,bhkd->bhqk", q, k) * (Dh ** -0.5)
        p = _softmax(scores, axis=-1)
        o = jnp.einsum("bhqk,bhkd->bhqd", p, v)
        return (lambda x, *d: x.transpose(*d))(o, 0, 2, 1, 3).reshape(B, Sq, Hq * Dh) @ wo

    def _B_ref(x, w1, w3, w2):
        gate = jnp.einsum("bsd,df->bsf", x, w1)
        up = jnp.einsum("bsd,df->bsf", x, w3)
        h = _silu(gate) * up
        out = jnp.einsum("bsf,fd->bsd", h, w2)
        return out

    x = A_x
    h = x + _A_ref(_layernorm(x, axis=-1), A_k_cache, A_v_cache, A_wq, A_wo)
    h2 = h + _B_ref(_layernorm(h, axis=-1), B_w1, B_w3, B_w2)
    return h2
```

```python
import jax
import jax.numpy as jnp
import numpy as np
from jax import lax
import jax.experimental.pallas as pl
import jax.experimental.pallas.tpu as pltpu

H, DH, SK, D, F = 32, 192, 32768, 640, 1536
W = min(4096, max(256, SK // 4))
BF = jnp.bfloat16
F32 = jnp.float32


def _bf16_round(v):
    u = int(np.float32(v).view(np.uint32))
    u = (u + 0x7FFF + ((u >> 16) & 1)) & 0xFFFF0000
    return float(np.uint32(u).view(np.float32))


SCALE = _bf16_round(DH ** -0.5)
EPS = _bf16_round(1e-5)


def _r(x):
    return x.astype(BF).astype(F32)


def _layernorm(x32):
    m = jnp.mean(x32, axis=-1, keepdims=True)
    c = x32 - m
    v = jnp.mean(c * c, axis=-1, keepdims=True)
    num = _r(x32 - _r(m))
    den = _r(jnp.sqrt(_r(_r(v) + EPS)))
    return (num / den).astype(BF)


def _merge(a, b):
    out, ia, ib = [], 0, 0
    while ia < len(a) or ib < len(b):
        if ib >= len(b) or (ia < len(a) and ia * len(b) <= ib * len(a)):
            out.append(a[ia])
            ia += 1
        else:
            out.append(b[ib])
            ib += 1
    return out


def _two_threads(a, b):
    return _merge([(p, 0) for p in a], [(p, 1) for p in b])


def make_kernel(R=3, kv_piece=(32, 512), GQ=5, wq_g=3, GO=8, wo_piece=(1, 16), G13=4, G2=4, w2_rows=16,
                w2ch=(128, 128, 128), nq=2, n0=400, tail=(64, 56), gsplit=(16, 16), dbg=()):
    RQ, RO, R13, R2 = D // GQ, H * DH // GO, D // G13, F // G2
    HPG = H // GO
    N2 = len(w2ch)
    w2off = [sum(w2ch[:i]) for i in range(N2)]
    assert sum(w2ch) == R2

    pr, pc = kv_piece
    kvp = _two_threads(*[[((r, pr), (c, pc)) for c in range(0, W, pc) for r in range(r0, r0 + DH // 2, pr)]
                         for r0 in (0, DH // 2)])
    wqp = [((g, min(wq_g, GQ - g)), (r, 8), (c, 512))
           for r in range(0, RQ, 8) for c in range(0, H * DH, 512) for g in range(0, GQ, wq_g)]
    wqp = _two_threads(wqp[:len(wqp) // 2], wqp[len(wqp) // 2:])
    wop = [((g, wo_piece[0]), (r, wo_piece[1]), (0, D))
           for r in range(0, RO, wo_piece[1]) for g in range(0, GO, wo_piece[0])]
    wop = [(p, (i // 2) % 2) for i, p in enumerate(wop)]
    w13p = [((0, G13), (r, 8), (c, 512)) for r in range(0, R13, 8) for c in range(0, F, 512)]
    w2p = [[((g, 1), (r, w2_rows), (0, D)) for r in range(w2off[c], w2off[c] + w2ch[c], w2_rows) for g in range(G2)]
           for c in range(N2)]

    def kernel(x_hbm, kt_hbm, vt_hbm, wq_hbm, wo_hbm, w1_hbm, w3_hbm, w2_hbm, o_hbm,
               x_v, wq_v, q_v, p_v, ring, wo_v, w1_v, w3_v, w2_v, o_v, sem_o):

        def body(sem_x, sem_f, sem_wq, sem_kv, sem_wo, sem_w13, sem_w2):
            def issue(jobs):
                for (src, dst, sem, p, thread) in jobs:
                    idx = tuple(pl.ds(*d) for d in p)
                    pltpu.make_async_copy(src.at[idx], dst.at[idx], sem).start(priority=thread)

            def wait_all(ref, sem):
                pltpu.make_async_copy(ref, ref, sem).wait()

            def block_jobs(src_hbm, h, slot):
                src = src_hbm.at[h, :, pl.ds(SK - W, W)]
                return [(src, ring.at[slot], sem_kv.at[slot], p, t) for p, t in kvp]

            x_copy = pltpu.make_async_copy(x_hbm, x_v, sem_x)
            x_copy.start()
            issue([(wq_hbm, wq_v, sem_f if p[1][0] == 0 else sem_wq, p, t) for p, t in wqp])
            wait_all(wq_v.at[:, pl.ds(0, 8)], sem_f)
            jobs = [(wo_hbm, wo_v, sem_wo, p, t) for p, t in wop]
            for h in range(R):
                jobs += block_jobs(kt_hbm, h, h)
            issue(jobs[:n0])

            x_copy.wait()
            x32 = x_v[...].astype(F32)
            lnx = jnp.broadcast_to(_layernorm(x32), (8, D))
            wait_all(wq_v.at[:, pl.ds(8, RQ - 8)], sem_wq)
            QC = H // nq
            rest = jobs[n0:]
            for c in range(nq):
                wq_c = wq_v[:, :, c * QC * DH:(c + 1) * QC * DH].reshape(D, QC * DH)
                qc = jnp.dot(lnx, wq_c, preferred_element_type=F32)
                for j in range(QC):
                    q_v[c * QC + j] = qc[:, j * DH:(j + 1) * DH]
                issue(rest[c * len(rest) // nq:(c + 1) * len(rest) // nq])
            wait_all(wo_v, sem_wo)

            def scores(h, slot):
                wait_all(ring.at[slot], sem_kv.at[slot])
                s = jnp.dot(q_v[h].astype(BF), ring[slot], preferred_element_type=F32)
                s = _r(_r(s) * SCALE)
                m = jnp.max(s, axis=-1, keepdims=True)
                e = _r(jnp.exp(_r(s - m)))
                l = _r(jnp.sum(e, axis=-1, keepdims=True))
                p_v[h] = e / l

            def k_step(h, _):
                slot = h % R
                scores(h, slot)
                issue(block_jobs(kt_hbm, h + R, slot))
                return _

            lax.fori_loop(0, H - R, k_step, 0)

            def kv_step(h, _):
                slot = h % R
                scores(h, slot)
                issue(block_jobs(vt_hbm, h + R - H, slot))
                return _

            lax.fori_loop(H - R, H, kv_step, 0)

            def values(h, slot, attn):
                wait_all(ring.at[slot], sem_kv.at[slot])
                o = lax.dot_general(p_v[h].astype(BF), ring[slot], (((1,), (1,)), ((), ())),
                                    preferred_element_type=F32)
                row = (h % HPG) * DH
                if not isinstance(h, int):
                    row = pl.multiple_of(row, DH)
                return attn + jnp.dot(o.astype(BF), wo_v[h // HPG, pl.ds(row, DH), :],
                                      preferred_element_type=F32)

            def v_step(h, attn):
                slot = (h + H) % R
                attn = values(h, slot, attn)
                issue(block_jobs(vt_hbm, h + R, slot))
                return attn

            attn = lax.fori_loop(0, H - R, v_step, jnp.zeros((8, D), F32))

            wj = []
            for p in w13p:
                wj += [(w1_hbm, w1_v, sem_w13, p, 0), (w3_hbm, w3_v, sem_w13, p, 1)]
            for c in range(N2):
                wj += [(w2_hbm, w2_v, sem_w2.at[c], p, i % 2) for i, p in enumerate(w2p[c])]
            cuts = [0]
            for n in tail:
                cuts.append(cuts[-1] + n)
            cuts = cuts + [len(wj) - sum(gsplit)] * (R + 1 - len(cuts))
            for i, h in enumerate(range(H - R, H)):
                attn = values(h, (h + H) % R, attn)
                issue(wj[cuts[i]:cuts[i + 1]])
            pos = cuts[R]
            hres = _r(x32 + _r(attn))
            lnh = _layernorm(hres)
            wait_all(w1_v, sem_w13)
            wait_all(w3_v, sem_w13)
            gate = _r(jnp.dot(lnh, w1_v[...].reshape(D, F), preferred_element_type=F32))
            issue(wj[pos:pos + gsplit[0]])
            up = _r(jnp.dot(lnh, w3_v[...].reshape(D, F), preferred_element_type=F32))
            issue(wj[pos + gsplit[0]:])
            hm = _r(_r(gate * _r(jax.nn.sigmoid(gate))) * up)
            out = None
            for c in range(N2):
                r0, nr = w2off[c], w2ch[c]
                hc = jnp.concatenate([hm[:, g * R2 + r0:g * R2 + r0 + nr] for g in range(G2)], axis=1).astype(BF)
                wait_all(w2_v.at[:, pl.ds(r0, nr)], sem_w2.at[c])
                if "notail" in dbg and c == N2 - 1:
                    continue
                o_ = jnp.dot(hc, w2_v[:, r0:r0 + nr, :].reshape(G2 * nr, D), preferred_element_type=F32)
                out = o_ if out is None else out + o_
            res = hres + _r(out)
            o_v[...] = res[0:1, :].astype(o_v.dtype)
            pltpu.make_async_copy(o_v, o_hbm, sem_o).start()

        dma = pltpu.SemaphoreType.DMA
        pl.run_scoped(body, dma(()), dma(()), dma(()), dma((R,)), dma(()), dma(()), dma((N2,)))
        pltpu.make_async_copy(o_v, o_hbm, sem_o).wait()

    @jax.jit
    def run(A_x, A_k_cache, A_v_cache, A_wq, A_wo, B_x, B_w1, B_w3, B_w2):
        del B_x
        x = A_x.reshape(1, D)
        kt = jnp.swapaxes(A_k_cache.reshape(H, SK, DH), 1, 2)
        vt = jnp.swapaxes(A_v_cache.reshape(H, SK, DH), 1, 2)
        out = pl.pallas_call(
            kernel,
            out_shape=jax.ShapeDtypeStruct((1, D), A_x.dtype),
            in_specs=[pl.BlockSpec(memory_space=pl.ANY)] * 8,
            out_specs=pl.BlockSpec(memory_space=pl.ANY),
            scratch_shapes=[
                pltpu.VMEM((1, D), BF),
                pltpu.VMEM((GQ, RQ, H * DH), BF),
                pltpu.VMEM((H, 8, DH), F32),
                pltpu.VMEM((H, 8, W), F32),
                pltpu.VMEM((R, DH, W), BF),
                pltpu.VMEM((GO, RO, D), BF),
                pltpu.VMEM((G13, R13, F), BF),
                pltpu.VMEM((G13, R13, F), BF),
                pltpu.VMEM((G2, R2, D), BF),
                pltpu.VMEM((1, D), BF),
                pltpu.SemaphoreType.DMA(()),
            ],
            compiler_params=pltpu.CompilerParams(vmem_limit_bytes=64 * 1024 * 1024),
        )(x, kt, vt, A_wq.reshape(GQ, RQ, H * DH), A_wo.reshape(GO, RO, D),
          B_w1.reshape(G13, R13, F), B_w3.reshape(G13, R13, F), B_w2.reshape(G2, R2, D))
        return out.reshape(1, 1, D)

    return run


pallas_sequential_preLN__sliding_block_cached__glu_gated_swiglu__decode_kernel = make_kernel()
```

```python
import jax
import jax.numpy as jnp
import numpy as np
from jax import lax
import jax.experimental.pallas as pl
import jax.experimental.pallas.tpu as pltpu

H, DH, SK, D, F = 32, 192, 32768, 640, 1536
W = min(4096, max(256, SK // 4))
BF = jnp.bfloat16
F32 = jnp.float32


def _bf16_round(v):
    u = int(np.float32(v).view(np.uint32))
    u = (u + 0x7FFF + ((u >> 16) & 1)) & 0xFFFF0000
    return float(np.uint32(u).view(np.float32))


SCALE = _bf16_round(DH ** -0.5)
EPS = _bf16_round(1e-5)


def _r(x):
    return x.astype(BF).astype(F32)


def _layernorm(x32):
    m = jnp.mean(x32, axis=-1, keepdims=True)
    c = x32 - m
    v = jnp.mean(c * c, axis=-1, keepdims=True)
    num = _r(x32 - _r(m))
    den = _r(jnp.sqrt(_r(_r(v) + EPS)))
    return (num / den).astype(BF)


def _merge(a, b):
    out, ia, ib = [], 0, 0
    while ia < len(a) or ib < len(b):
        if ib >= len(b) or (ia < len(a) and ia * len(b) <= ib * len(a)):
            out.append(a[ia])
            ia += 1
        else:
            out.append(b[ib])
            ib += 1
    return out


def _two_threads(a, b):
    return _merge([(p, 0) for p in a], [(p, 1) for p in b])


def make_kernel(R=4, NC=4, kv_piece=(32, 512), GQ=4, wq_piece=(2, 1024), wq_phases=3, GO=8, wo_piece=(1, 16), G13=4, G2=4, w2_rows=(16,) * 5, w2th=('1010', '1010', '1111', '1111'),
                w2ch=(192, 96, 64, 32), nq=2, n0=400, tail=(8, 8, 4), w13ch=(96, 64), gsplit=(1, 4), kv1=1, fq=0, fo=0, f13=0, ksh=0, dbg=()):
    RQ, RO, R13, R2 = D // GQ, H * DH // GO, D // G13, F // G2
    HPG = H // GO
    N2 = len(w2ch)
    w2off = [sum(w2ch[:i]) for i in range(N2)]
    w13off = [sum(w13ch[:i]) for i in range(len(w13ch))]
    assert sum(w2ch) == R2 and sum(w13ch) == R13

    pr, pc = kv_piece
    kvp = _two_threads(*[[((r, pr), (c, pc)) for c in range(0, W, pc) for r in range(r0, r0 + DH // 2, pr)]
                         for r0 in (0, DH // 2)])
    if kv1:
        kvp = [kvp[i ^ 1] for i in range(len(kvp))]
    chunks = [(r, c) for r in range(0, RQ, 8) for c in range(0, H * DH, wq_piece[1])]
    ny = len(chunks) // wq_phases
    wqp = [((g, wq_piece[0]), (chunks[j * ny + y][0], 8), (chunks[j * ny + y][1], wq_piece[1]))
           for y in range(ny) for j in range(wq_phases) for g in range(0, GQ, wq_piece[0])]
    wqp = [(p, (i + (fq & 1)) % 2) for i, p in enumerate(wqp)]
    if fq & 2:
        wqp = [wqp[i ^ 1] for i in range(len(wqp))]
    wop = [((g, wo_piece[0]), (r, wo_piece[1]), (0, D))
           for r in range(0, RO, wo_piece[1]) for g in range(0, GO, wo_piece[0])]
    wop = [(p, (i // 2 + (fo & 1)) % 2) for i, p in enumerate(wop)]
    if fo & 2:
        wop = [wop[i ^ 2] for i in range(len(wop))]

    def kernel(x_hbm, kt_hbm, vt_hbm, wq_hbm, wo_hbm, w1_hbm, w3_hbm, w2_hbm, o_hbm,
               x_v, wq_v, q_v, p_v, ring, wo_v, w1_v, w3_v, w2_v, o_v, sem_o):

        def body(sem_x, sem_f, sem_wq, sem_kv, sem_wo, sem_w13, sem_w2):
            def issue(jobs):
                for (src, dst, sem, p, thread) in jobs:
                    idx = tuple(pl.ds(*d) for d in p)
                    pltpu.make_async_copy(src.at[idx], dst.at[idx], sem).start(priority=thread)

            def wait_all(ref, sem):
                pltpu.make_async_copy(ref, ref, sem).wait()

            def block_jobs(src_hbm, h, slot):
                src = src_hbm.at[h, :, pl.ds(SK - W, W)]
                return [(src, ring.at[slot], sem_kv.at[slot], p, t) for p, t in kvp]

            x_copy = pltpu.make_async_copy(x_hbm, x_v, sem_x)
            x_copy.start()
            issue([(wq_hbm, wq_v, sem_f if p[1][0] == 0 else sem_wq, p, t) for p, t in wqp])
            wait_all(wq_v.at[:, pl.ds(0, 8)], sem_f)
            jobs = [(wo_hbm, wo_v, sem_wo, p, t) for p, t in wop]
            for h in range(R):
                jobs += block_jobs(kt_hbm, h, h)
            issue(jobs[:n0])

            x_copy.wait()
            x32 = x_v[...].astype(F32)
            lnx = jnp.broadcast_to(_layernorm(x32), (8, D))
            wait_all(wq_v.at[:, pl.ds(8, RQ - 8)], sem_wq)
            QC = H // nq
            rest = jobs[n0:]
            for c in range(nq):
                if "noq" in dbg:
                    issue(rest[c * len(rest) // nq:(c + 1) * len(rest) // nq])
                    continue
                wq_c = wq_v[:, :, c * QC * DH:(c + 1) * QC * DH].reshape(D, QC * DH)
                qc = jnp.dot(lnx, wq_c, preferred_element_type=F32)
                for j in range(QC):
                    q_v[c * QC + j] = qc[:, j * DH:(j + 1) * DH]
                issue(rest[c * len(rest) // nq:(c + 1) * len(rest) // nq])
            wait_all(wo_v, sem_wo)

            CW = W // NC

            def parts(jobs, n):
                return [jobs[i * len(jobs) // n:(i + 1) * len(jobs) // n] for i in range(n)]

            def scores(h, slot, jobs):
                wait_all(ring.at[slot], sem_kv.at[slot])
                qh = q_v[h].astype(BF)
                s = []
                for c, part in enumerate(parts(jobs, NC)):
                    if "nok" not in dbg:
                        s.append(jnp.dot(qh, ring[slot, :, c * CW:(c + 1) * CW], preferred_element_type=F32))
                    issue(part)
                if "nok" in dbg:
                    return
                s = _r(_r(jnp.concatenate(s, axis=1)) * SCALE)
                m = jnp.max(s, axis=-1, keepdims=True)
                e = _r(jnp.exp(_r(s - m)))
                l = _r(jnp.sum(e, axis=-1, keepdims=True))
                p_v[h] = e / l

            scores(0, 0, [])

            def k_step(h, _):
                scores(h, h % R, block_jobs(kt_hbm, h + R - 1, (h - 1) % R))
                return _

            lax.fori_loop(1, H - R + 1, k_step, 0)

            def kv_step(h, _):
                scores(h, h % R, block_jobs(vt_hbm, h + R - 1 - H, (h - 1) % R))
                return _

            lax.fori_loop(H - R + 1, H, kv_step, 0)

            def values(h, slot, attn, jobs):
                wait_all(ring.at[slot], sem_kv.at[slot])
                o = None
                for c, part in enumerate(parts(jobs, NC)):
                    if "nov" not in dbg:
                        o_ = lax.dot_general(p_v[h, :, c * CW:(c + 1) * CW].astype(BF),
                                             ring[slot, :, c * CW:(c + 1) * CW],
                                             (((1,), (1,)), ((), ())), preferred_element_type=F32)
                        o = o_ if o is None else o + o_
                    issue(part)
                if "nov" in dbg:
                    return attn
                row = (h % HPG) * DH
                if not isinstance(h, int):
                    row = pl.multiple_of(row, DH)
                return attn + jnp.dot(o.astype(BF), wo_v[h // HPG, pl.ds(row, DH), :],
                                      preferred_element_type=F32)

            def v_step(h, attn):
                return values(h, (h + H) % R, attn, block_jobs(vt_hbm, h + R - 1, (h + H - 1) % R))

            attn = lax.fori_loop(0, H - R + 1, v_step, jnp.zeros((8, D), F32))

            def chunk_of(r, offsets):
                return sum((r >= o).astype(jnp.int32) for o in offsets[1:])

            def issue_w13(lo, hi):
                def step(i, _):
                    r = pl.multiple_of(i * 8, 8)
                    sem = sem_w13.at[chunk_of(r, w13off)]
                    for c in range(0, F, 512):
                        idx = (slice(None), pl.ds(r, 8), pl.ds(c, 512))
                        two = [(w1_hbm, w1_v, f13 & 1), (w3_hbm, w3_v, 1 - (f13 & 1))]
                        for src, dst, t in (two[::-1] if f13 & 2 else two):
                            pltpu.make_async_copy(src.at[idx], dst.at[idx], sem).start(priority=t)
                    return _
                if hi > lo:
                    lax.fori_loop(lo, hi, step, 0)

            def issue_w2(lo, hi):
                for c in range(lo, hi):
                    def step(i, _, c=c):
                        r = pl.multiple_of(w2off[c] + i * w2_rows[c], w2_rows[c])
                        for g in range(G2):
                            idx = (g, pl.ds(r, w2_rows[c]))
                            pltpu.make_async_copy(w2_hbm.at[idx], w2_v.at[idx], sem_w2.at[c]).start(priority=int(w2th[c][g]))
                        return _
                    lax.fori_loop(0, w2ch[c] // w2_rows[c], step, 0)

            pos = 0
            for n, h in zip(tail, range(H - R + 1, H), strict=True):
                issue_w13(pos, pos + n)
                attn = values(h, (h + H) % R, attn, [])
                pos += n
            issue_w13(pos, R13 // 8)
            hres = _r(x32 + _r(attn))
            lnh = _layernorm(hres).astype(F32)

            def columns(v, group, r0, nr):
                return jnp.concatenate([v[:, g + r0:g + r0 + nr] for g in range(0, v.shape[1], group)], axis=1).astype(BF)

            gate = up = None
            pos = 0
            for c, (r0, nr) in enumerate(zip(w13off, w13ch)):
                lc = columns(lnh, R13, r0, nr)
                issue_w2(pos, gsplit[c])
                pos = gsplit[c]
                wait_all(w1_v.at[:, pl.ds(r0, nr)], sem_w13.at[c])
                wait_all(w3_v.at[:, pl.ds(r0, nr)], sem_w13.at[c])
                g_ = jnp.dot(lc, w1_v[:, r0:r0 + nr, :].reshape(G13 * nr, F), preferred_element_type=F32)
                u_ = jnp.dot(lc, w3_v[:, r0:r0 + nr, :].reshape(G13 * nr, F), preferred_element_type=F32)
                gate = g_ if gate is None else gate + g_
                up = u_ if up is None else up + u_
            issue_w2(pos, N2)
            gate, up = _r(gate), _r(up)
            hm = _r(_r(gate * _r(jax.nn.sigmoid(gate))) * up)
            out = None
            for c in range(N2):
                r0, nr = w2off[c], w2ch[c]
                hc = columns(hm, R2, r0, nr)
                wait_all(w2_v.at[:, pl.ds(r0, nr)], sem_w2.at[c])
                if "notail" in dbg and c == N2 - 1:
                    continue
                o_ = jnp.dot(hc, w2_v[:, r0:r0 + nr, :].reshape(G2 * nr, D), preferred_element_type=F32)
                out = o_ if out is None else out + o_
            res = hres + _r(out)
            o_v[...] = res[0:1, :].astype(o_v.dtype)
            pltpu.make_async_copy(o_v, o_hbm, sem_o).start()

        dma = pltpu.SemaphoreType.DMA
        pl.run_scoped(body, dma(()), dma(()), dma(()), dma((R,)), dma(()), dma((len(w13ch),)), dma((N2,)))
        pltpu.make_async_copy(o_v, o_hbm, sem_o).wait()

    @jax.jit
    def run(A_x, A_k_cache, A_v_cache, A_wq, A_wo, B_x, B_w1, B_w3, B_w2):
        del B_x
        x = A_x.reshape(1, D)
        kt = jnp.swapaxes(A_k_cache.reshape(H, SK, DH), 1, 2)
        vt = jnp.swapaxes(A_v_cache.reshape(H, SK, DH), 1, 2)
        out = pl.pallas_call(
            kernel,
            out_shape=jax.ShapeDtypeStruct((1, D), A_x.dtype),
            in_specs=[pl.BlockSpec(memory_space=pl.ANY)] * 8,
            out_specs=pl.BlockSpec(memory_space=pl.ANY),
            scratch_shapes=[
                pltpu.VMEM((1, D), BF),
                pltpu.VMEM((GQ, RQ, H * DH), BF),
                pltpu.VMEM((H, 8, DH), F32),
                pltpu.VMEM((H, 8, W), F32),
                pltpu.VMEM((R, DH, W), BF),
                pltpu.VMEM((GO, RO, D), BF),
                pltpu.VMEM((G13, R13, F), BF),
                pltpu.VMEM((G13, R13, F), BF),
                pltpu.VMEM((G2, R2, D), BF),
                pltpu.VMEM((1, D), BF),
                pltpu.SemaphoreType.DMA(()),
            ],
            compiler_params=pltpu.CompilerParams(vmem_limit_bytes=64 * 1024 * 1024),
        )(x, kt, vt, A_wq.reshape(GQ, RQ, H * DH), A_wo.reshape(GO, RO, D),
          B_w1.reshape(G13, R13, F), B_w3.reshape(G13, R13, F), B_w2.reshape(G2, R2, D))
        return out.reshape(1, 1, D)

    return run


pallas_sequential_preLN__sliding_block_cached__glu_gated_swiglu__decode_kernel = make_kernel()
```

```python
import jax
import jax.numpy as jnp
import numpy as np
from jax import lax
import jax.experimental.pallas as pl
import jax.experimental.pallas.tpu as pltpu

H, DH, SK, D, F = 32, 192, 32768, 640, 1536
W = min(4096, max(256, SK // 4))
BF = jnp.bfloat16
F32 = jnp.float32


def _bf16_round(v):
    u = int(np.float32(v).view(np.uint32))
    u = (u + 0x7FFF + ((u >> 16) & 1)) & 0xFFFF0000
    return float(np.uint32(u).view(np.float32))


SCALE = _bf16_round(DH ** -0.5)
EPS = _bf16_round(1e-5)


def _r(x):
    return x.astype(BF).astype(F32)


def _layernorm(x32):
    m = jnp.mean(x32, axis=-1, keepdims=True)
    c = x32 - m
    v = jnp.mean(c * c, axis=-1, keepdims=True)
    num = _r(x32 - _r(m))
    den = _r(jnp.sqrt(_r(_r(v) + EPS)))
    return (num / den).astype(BF)


def make_kernel(R=4, kv_rows=32, kv_order=((5, 0), (4, 1), (3, 2)), tail=(60, 60, 0),
                w2ch=(128, 128, 96, 32), w2th=("1010", "1010", "1111", "1111")):
    GQ, GO, G13, G2 = 4, 8, 4, 4
    RQ, RO, R13, R2 = D // GQ, H * DH // GO, D // G13, F // G2
    HPG = H // GO
    N2 = len(w2ch)
    w2off = [sum(w2ch[:i]) for i in range(N2)]
    assert sum(w2ch) == R2 and H % R == 0

    kvp = [(((i * kv_rows, kv_rows), (c, 512)), t)
           for c in range(0, W, 512) for pair in kv_order for i, t in zip(pair, (1, 0))]
    runs = [(r, c) for r in range(0, RQ, 8) for c in range(0, H * DH, 1024)]
    ny = len(runs) // 3
    wqp = [(((g, 2), (runs[j * ny + y][0], 8), (runs[j * ny + y][1], 1024)), g // 2)
           for y in range(ny) for j in range(3) for g in (0, 2)]
    wop = [(((g, 1), (r, 16), (0, D)), g // 2 % 2) for r in range(0, RO, 16) for g in range(GO)]
    w13p = [((0, G13), (r, 8), (c, 512)) for r in range(0, R13, 8) for c in range(0, F, 512)]

    def kernel(x_hbm, kt_hbm, vt_hbm, wq_hbm, wo_hbm, w1_hbm, w3_hbm, w2_hbm, o_hbm,
               x_v, wq_v, q_v, p_v, ring, wo_v, w1_v, w3_v, w2_v, hb_v, o_v, sem_o):

        def body(sem_x, sem_f, sem_wq, sem_kv, sem_wo, sem_w13, sem_w2):
            def issue(jobs):
                for (src, dst, sem, p, thread) in jobs:
                    idx = tuple(pl.ds(*d) for d in p)
                    pltpu.make_async_copy(src.at[idx], dst.at[idx], sem).start(priority=thread)

            def wait_all(ref, sem):
                pltpu.make_async_copy(ref, ref, sem).wait()

            def block_jobs(src_hbm, h, slot):
                src = src_hbm.at[h, :, pl.ds(SK - W, W)]
                return [(src, ring.at[slot], sem_kv.at[slot], p, t) for p, t in kvp]

            x_copy = pltpu.make_async_copy(x_hbm, x_v, sem_x)
            x_copy.start()
            issue([(wq_hbm, wq_v, sem_f if p[1][0] == 0 else sem_wq, p, t) for p, t in wqp])
            wait_all(wq_v.at[:, pl.ds(0, 8)], sem_f)
            issue([(wo_hbm, wo_v, sem_wo, p, t) for p, t in wop])

            x_copy.wait()
            x32 = x_v[...].astype(F32)
            lnx = jnp.broadcast_to(_layernorm(x32), (8, D))
            wait_all(wq_v.at[:, pl.ds(8, RQ - 8)], sem_wq)
            QC = H // R

            def q_step(i, _):
                wq_c = wq_v[:, :, pl.ds(pl.multiple_of(i * (QC * DH), 128), QC * DH)].reshape(D, QC * DH)
                qc = jnp.dot(lnx, wq_c, preferred_element_type=F32)
                for j in range(QC):
                    q_v[i * QC + j] = qc[:, j * DH:(j + 1) * DH]
                issue(block_jobs(kt_hbm, i, i))
                return _

            lax.fori_loop(0, R, q_step, 0)
            wait_all(wo_v, sem_wo)

            def scores(h, slot, jobs):
                wait_all(ring.at[slot], sem_kv.at[slot])
                s = jnp.dot(q_v[h].astype(BF), ring[slot], preferred_element_type=F32)
                issue(jobs)
                s = _r(_r(s) * SCALE)
                m = jnp.max(s, axis=-1, keepdims=True)
                e = _r(jnp.exp(_r(s - m)))
                l = _r(jnp.sum(e, axis=-1, keepdims=True))
                p_v[h] = e / l

            def k_step(h, _):
                scores(h, h % R, block_jobs(kt_hbm, h + R - 1, (h - 1) % R))
                return _

            def kv_step(h, _):
                scores(h, h % R, block_jobs(vt_hbm, h + R - 1 - H, (h - 1) % R))
                return _

            scores(0, 0, [])
            lax.fori_loop(1, H - R + 1, k_step, 0)
            lax.fori_loop(H - R + 1, H, kv_step, 0)

            def values(h, slot, attn, jobs):
                wait_all(ring.at[slot], sem_kv.at[slot])
                o = lax.dot_general(p_v[h].astype(BF), ring[slot], (((1,), (1,)), ((), ())),
                                    preferred_element_type=F32)
                issue(jobs)
                row = (h % HPG) * DH
                if not isinstance(h, int):
                    row = pl.multiple_of(row, DH)
                return attn + jnp.dot(o.astype(BF), wo_v[h // HPG, pl.ds(row, DH), :],
                                      preferred_element_type=F32)

            def v_step(h, attn):
                return values(h, h % R, attn, block_jobs(vt_hbm, h + R - 1, (h + R - 1) % R))

            attn = lax.fori_loop(0, H - R + 1, v_step, jnp.zeros((8, D), F32))

            w13_jobs = [(src, dst, sem_w13, p, t)
                        for p in w13p for src, dst, t in ((w1_hbm, w1_v, 0), (w3_hbm, w3_v, 1))]
            assert sum(tail) == len(w13_jobs)
            pos = 0
            for n, h in zip(tail, range(H - R + 1, H), strict=True):
                attn = values(h, h % R, attn, w13_jobs[pos:pos + n])
                pos += n
            for c in range(N2):
                def w2_step(i, _, c=c):
                    r = pl.multiple_of(w2off[c] + i * 16, 16)
                    for g in range(G2):
                        idx = (g, pl.ds(r, 16))
                        pltpu.make_async_copy(w2_hbm.at[idx], w2_v.at[idx], sem_w2.at[c]).start(priority=int(w2th[c][g]))
                    return _

                lax.fori_loop(0, w2ch[c] // 16, w2_step, 0)

            def columns(v, r0, nr):
                return jnp.concatenate([v[:, g + r0:g + r0 + nr] for g in range(0, F, R2)], axis=1).astype(BF)

            hres = _r(x32 + _r(attn))
            lnh = _layernorm(hres)
            wait_all(w1_v, sem_w13)
            wait_all(w3_v, sem_w13)
            gate = _r(jnp.dot(lnh, w1_v[...].reshape(D, F), preferred_element_type=F32))
            up = _r(jnp.dot(lnh, w3_v[...].reshape(D, F), preferred_element_type=F32))
            hm = _r(_r(gate * _r(jax.nn.sigmoid(gate))) * up)
            hcols = [columns(hm, w2off[c], w2ch[c]) for c in range(N2)]
            hb_v[...] = jnp.broadcast_to(hcols[-1][0:1].astype(F32), (128, G2 * w2ch[-1])).T
            out = None
            for c in range(N2 - 1):
                r0, nr = w2off[c], w2ch[c]
                wait_all(w2_v.at[:, pl.ds(r0, nr)], sem_w2.at[c])
                o_ = jnp.dot(hcols[c], w2_v[:, r0:r0 + nr, :].reshape(G2 * nr, D), preferred_element_type=F32)
                out = o_ if out is None else out + o_
            r0, nr = w2off[-1], w2ch[-1]
            wait_all(w2_v.at[:, pl.ds(r0, nr)], sem_w2.at[N2 - 1])
            last = [jnp.sum(w2_v[:, r0:r0 + nr, n:n + 128].reshape(G2 * nr, 128).astype(F32) * hb_v[...],
                            axis=0, keepdims=True) for n in range(0, D, 128)]
            out = out[0:1] + jnp.concatenate(last, axis=1)
            o_v[...] = (hres[0:1] + _r(out)).astype(o_v.dtype)
            pltpu.make_async_copy(o_v, o_hbm, sem_o).start()

        dma = pltpu.SemaphoreType.DMA
        pl.run_scoped(body, dma(()), dma(()), dma(()), dma((R,)), dma(()), dma(()), dma((N2,)))
        pltpu.make_async_copy(o_v, o_hbm, sem_o).wait()

    @jax.jit
    def run(A_x, A_k_cache, A_v_cache, A_wq, A_wo, B_x, B_w1, B_w3, B_w2):
        del B_x
        x = A_x.reshape(1, D)
        kt = jnp.swapaxes(A_k_cache.reshape(H, SK, DH), 1, 2)
        vt = jnp.swapaxes(A_v_cache.reshape(H, SK, DH), 1, 2)
        out = pl.pallas_call(
            kernel,
            out_shape=jax.ShapeDtypeStruct((1, D), A_x.dtype),
            in_specs=[pl.BlockSpec(memory_space=pl.ANY)] * 8,
            out_specs=pl.BlockSpec(memory_space=pl.ANY),
            scratch_shapes=[
                pltpu.VMEM((1, D), BF),
                pltpu.VMEM((GQ, RQ, H * DH), BF),
                pltpu.VMEM((H, 8, DH), F32),
                pltpu.VMEM((H, 8, W), F32),
                pltpu.VMEM((R, DH, W), BF),
                pltpu.VMEM((GO, RO, D), BF),
                pltpu.VMEM((G13, R13, F), BF),
                pltpu.VMEM((G13, R13, F), BF),
                pltpu.VMEM((G2, R2, D), BF),
                pltpu.VMEM((G2 * w2ch[-1], 128), F32),
                pltpu.VMEM((1, D), BF),
                pltpu.SemaphoreType.DMA(()),
            ],
            compiler_params=pltpu.CompilerParams(vmem_limit_bytes=64 * 1024 * 1024),
        )(x, kt, vt, A_wq.reshape(GQ, RQ, H * DH), A_wo.reshape(GO, RO, D),
          B_w1.reshape(G13, R13, F), B_w3.reshape(G13, R13, F), B_w2.reshape(G2, R2, D))
        return out.reshape(1, 1, D)

    return run


pallas_sequential_preLN__sliding_block_cached__glu_gated_swiglu__decode_kernel = make_kernel()
```

```python
import jax
import jax.numpy as jnp
import numpy as np
from jax import lax
import jax.experimental.pallas as pl
import jax.experimental.pallas.tpu as pltpu

H, DH, SK, D, F = 32, 192, 32768, 640, 1536
W = min(4096, max(256, SK // 4))
BF = jnp.bfloat16
F32 = jnp.float32


def _bf16_round(v):
    u = int(np.float32(v).view(np.uint32))
    u = (u + 0x7FFF + ((u >> 16) & 1)) & 0xFFFF0000
    return float(np.uint32(u).view(np.float32))


SCALE = _bf16_round(DH ** -0.5)
EPS = _bf16_round(1e-5)


def _r(x):
    return x.astype(BF).astype(F32)


def _layernorm(x32):
    m = jnp.mean(x32, axis=-1, keepdims=True)
    c = x32 - m
    v = jnp.mean(c * c, axis=-1, keepdims=True)
    num = _r(x32 - _r(m))
    den = _r(jnp.sqrt(_r(_r(v) + EPS)))
    return (num / den).astype(BF)


def make_kernel(R=4, kv_rows=32, kv_order=((3, 0), (4, 1), (5, 2)),
                w2ch=(128, 128, 96, 32), w2th=("1010", "1010", "1111", "1111")):
    GQ, GO, G13, G2 = 5, 8, 4, 4
    RQ, RO, R13, R2 = D // GQ, H * DH // GO, D // G13, F // G2
    HPG = H // GO
    N2 = len(w2ch)
    w2off = [sum(w2ch[:i]) for i in range(N2)]
    assert sum(w2ch) == R2 and H % R == 0

    kvp = [(((i * kv_rows, kv_rows), (c, 512)), t)
           for c in range(0, W, 512) for pair in kv_order for i, t in zip(pair, (1, 0))]
    runs = [(r, c) for r in range(0, RQ, 8) for c in range(0, H * DH, 512)]
    ny = len(runs) // 3
    wqp = [(((g, n), (runs[j * ny + y][0], 8), (runs[j * ny + y][1], 512)), t)
           for y in range(ny) for j in range(3) for g, n, t in ((0, 2, 0), (2, 3, 1))]
    wop = [(((g, 1), (r, 16), (0, D)), g // 2 % 2) for r in range(0, RO, 16) for g in range(GO)]
    w13p = [((0, G13), (r, 8), (c, 512)) for r in range(0, R13, 8) for c in range(0, F, 512)]

    def kernel(x_hbm, kt_hbm, vt_hbm, wq_hbm, wo_hbm, w1_hbm, w3_hbm, w2_hbm, o_hbm,
               x_v, wq_v, q_v, p_v, ring, wo_v, w1_v, w3_v, w2_v, hb_v, o_v, sem_o):

        def body(sem_x, sem_f, sem_wq, sem_kv, sem_wo, sem_w13, sem_w2):
            def issue(jobs):
                for (src, dst, sem, p, thread) in jobs:
                    idx = tuple(pl.ds(*d) for d in p)
                    pltpu.make_async_copy(src.at[idx], dst.at[idx], sem).start(priority=thread)

            def wait_all(ref, sem):
                pltpu.make_async_copy(ref, ref, sem).wait()

            def block_jobs(src_hbm, h, slot):
                src = src_hbm.at[h, :, pl.ds(SK - W, W)]
                return [(src, ring.at[slot], sem_kv.at[slot], p, t) for p, t in kvp]

            x_copy = pltpu.make_async_copy(x_hbm, x_v, sem_x)
            x_copy.start()
            issue([(wq_hbm, wq_v, sem_f if p[1][0] == 0 else sem_wq, p, t) for p, t in wqp])
            wait_all(wq_v.at[:, pl.ds(0, 8)], sem_f)
            issue([(wo_hbm, wo_v, sem_wo, p, t) for p, t in wop])

            x_copy.wait()
            x32 = x_v[...].astype(F32)
            lnx = jnp.broadcast_to(_layernorm(x32), (8, D))
            wait_all(wq_v.at[:, pl.ds(8, RQ - 8)], sem_wq)
            QC = H // R

            def q_step(i, _):
                wq_c = wq_v[:, :, pl.ds(pl.multiple_of(i * (QC * DH), 128), QC * DH)].reshape(D, QC * DH)
                qc = jnp.dot(lnx, wq_c, preferred_element_type=F32)
                for j in range(QC):
                    q_v[i * QC + j] = qc[:, j * DH:(j + 1) * DH]
                issue(block_jobs(kt_hbm, i, i))
                return _

            lax.fori_loop(0, R, q_step, 0)
            wait_all(wo_v, sem_wo)

            def scores(h, slot, jobs):
                wait_all(ring.at[slot], sem_kv.at[slot])
                s = jnp.dot(q_v[h].astype(BF), ring[slot], preferred_element_type=F32)
                issue(jobs)
                s = _r(_r(s) * SCALE)
                m = jnp.max(s, axis=-1, keepdims=True)
                e = _r(jnp.exp(_r(s - m)))
                l = _r(jnp.sum(e, axis=-1, keepdims=True))
                p_v[h] = e / l

            def k_step(h, _):
                scores(h, h % R, block_jobs(kt_hbm, h + R - 1, (h - 1) % R))
                return _

            def kv_step(h, _):
                scores(h, h % R, block_jobs(vt_hbm, h + R - 1 - H, (h - 1) % R))
                return _

            scores(0, 0, [])
            lax.fori_loop(1, H - R + 1, k_step, 0)
            lax.fori_loop(H - R + 1, H, kv_step, 0)

            def values(h, slot, attn, jobs):
                wait_all(ring.at[slot], sem_kv.at[slot])
                o = lax.dot_general(p_v[h].astype(BF), ring[slot], (((1,), (1,)), ((), ())),
                                    preferred_element_type=F32)
                issue(jobs)
                row = (h % HPG) * DH
                if not isinstance(h, int):
                    row = pl.multiple_of(row, DH)
                return attn + jnp.dot(o.astype(BF), wo_v[h // HPG, pl.ds(row, DH), :],
                                      preferred_element_type=F32)

            def v_step(h, attn):
                return values(h, h % R, attn, block_jobs(vt_hbm, h + R - 1, (h + R - 1) % R))

            attn = lax.fori_loop(0, H - R + 1, v_step, jnp.zeros((8, D), F32))

            w13_jobs = [(src, dst, sem_w13, p, t)
                        for p in w13p for src, dst, t in ((w1_hbm, w1_v, 0), (w3_hbm, w3_v, 1))]
            n13 = len(w13_jobs) // (R - 1)
            assert n13 * (R - 1) == len(w13_jobs)
            for i, h in enumerate(range(H - R + 1, H)):
                attn = values(h, h % R, attn, w13_jobs[i * n13:(i + 1) * n13])
            for c in range(N2):
                def w2_step(i, _, c=c):
                    r = pl.multiple_of(w2off[c] + i * 16, 16)
                    for g in range(G2):
                        idx = (g, pl.ds(r, 16))
                        pltpu.make_async_copy(w2_hbm.at[idx], w2_v.at[idx], sem_w2.at[c]).start(priority=int(w2th[c][g]))
                    return _

                lax.fori_loop(0, w2ch[c] // 16, w2_step, 0)

            def columns(v, r0, nr):
                return jnp.concatenate([v[:, g + r0:g + r0 + nr] for g in range(0, F, R2)], axis=1).astype(BF)

            hres = _r(x32 + _r(attn))
            lnh = _layernorm(hres)
            wait_all(w1_v, sem_w13)
            wait_all(w3_v, sem_w13)
            gate = _r(jnp.dot(lnh, w1_v[...].reshape(D, F), preferred_element_type=F32))
            up = _r(jnp.dot(lnh, w3_v[...].reshape(D, F), preferred_element_type=F32))
            hm = _r(_r(gate * _r(jax.nn.sigmoid(gate))) * up)
            hcols = [columns(hm, w2off[c], w2ch[c]) for c in range(N2)]
            hb_v[...] = jnp.broadcast_to(hcols[-1][0:1].astype(F32), (128, G2 * w2ch[-1])).T
            out = None
            for c in range(N2 - 1):
                r0, nr = w2off[c], w2ch[c]
                wait_all(w2_v.at[:, pl.ds(r0, nr)], sem_w2.at[c])
                o_ = jnp.dot(hcols[c], w2_v[:, r0:r0 + nr, :].reshape(G2 * nr, D), preferred_element_type=F32)
                out = o_ if out is None else out + o_
            r0, nr = w2off[-1], w2ch[-1]
            wait_all(w2_v.at[:, pl.ds(r0, nr)], sem_w2.at[N2 - 1])
            last = [jnp.sum(w2_v[:, r0:r0 + nr, n:n + 128].reshape(G2 * nr, 128).astype(F32) * hb_v[...],
                            axis=0, keepdims=True) for n in range(0, D, 128)]
            out = out[0:1] + jnp.concatenate(last, axis=1)
            o_v[...] = (hres[0:1] + _r(out)).astype(o_v.dtype)
            pltpu.make_async_copy(o_v, o_hbm, sem_o).start()

        dma = pltpu.SemaphoreType.DMA
        pl.run_scoped(body, dma(()), dma(()), dma(()), dma((R,)), dma(()), dma(()), dma((N2,)))
        pltpu.make_async_copy(o_v, o_hbm, sem_o).wait()

    @jax.jit
    def run(A_x, A_k_cache, A_v_cache, A_wq, A_wo, B_x, B_w1, B_w3, B_w2):
        del B_x
        x = A_x.reshape(1, D)
        kt = jnp.swapaxes(A_k_cache.reshape(H, SK, DH), 1, 2)
        vt = jnp.swapaxes(A_v_cache.reshape(H, SK, DH), 1, 2)
        out = pl.pallas_call(
            kernel,
            out_shape=jax.ShapeDtypeStruct((1, D), A_x.dtype),
            in_specs=[pl.BlockSpec(memory_space=pl.ANY)] * 8,
            out_specs=pl.BlockSpec(memory_space=pl.ANY),
            scratch_shapes=[
                pltpu.VMEM((1, D), BF),
                pltpu.VMEM((GQ, RQ, H * DH), BF),
                pltpu.VMEM((H, 8, DH), F32),
                pltpu.VMEM((H, 8, W), F32),
                pltpu.VMEM((R, DH, W), BF),
                pltpu.VMEM((GO, RO, D), BF),
                pltpu.VMEM((G13, R13, F), BF),
                pltpu.VMEM((G13, R13, F), BF),
                pltpu.VMEM((G2, R2, D), BF),
                pltpu.VMEM((G2 * w2ch[-1], 128), F32),
                pltpu.VMEM((1, D), BF),
                pltpu.SemaphoreType.DMA(()),
            ],
            compiler_params=pltpu.CompilerParams(vmem_limit_bytes=64 * 1024 * 1024),
        )(x, kt, vt, A_wq.reshape(GQ, RQ, H * DH), A_wo.reshape(GO, RO, D),
          B_w1.reshape(G13, R13, F), B_w3.reshape(G13, R13, F), B_w2.reshape(G2, R2, D))
        return out.reshape(1, 1, D)

    return run


pallas_sequential_preLN__sliding_block_cached__glu_gated_swiglu__decode_kernel = make_kernel()
```
